```python
import os as _os
_os.environ.setdefault("JAX_PLATFORMS", "cpu")
import jax
import jax.numpy as jnp

def _softmax(x, axis=-1):
    return jax.nn.softmax(x, axis=axis)
def _gelu(x):
    return jax.nn.gelu(x, approximate=True)
def _silu(x):
    return jax.nn.silu(x)
def _sigmoid(x):
    return jax.nn.sigmoid(x)
def _layernorm(x, axis=-1, eps=1e-5):
    m = jnp.mean(x, axis=axis, keepdims=True)
    v = jnp.var(x, axis=axis, keepdims=True)
    return (x - m) / jnp.sqrt(v + eps)
def _scatter_add(tgt, idx, src, axis=0):
    return tgt.at[idx].add(src)
def _segment_sum(src, seg, n):
    return jax.ops.segment_sum(src, seg, n)
class _Rng:
    def __init__(self, key):
        self._k = key
    def _next(self):
        self._k, sub = jax.random.split(self._k)
        return sub
    def normal(self, shape):
        return jax.random.normal(self._next(), shape, dtype=jnp.bfloat16)
    def randint(self, lo, hi, shape):
        return jax.random.randint(self._next(), shape, lo, hi, dtype=jnp.int32)
    def uniform(self, shape, lo=0.0, hi=1.0):
        return jax.random.uniform(self._next(), shape, jnp.bfloat16, lo, hi)
    def permutation(self, n):
        return jax.random.permutation(self._next(), n)


kernel_name = 'concat_heads__grouped_kv_mqa__sliding_block__prompt'

def setup_inputs():
    _rng = _Rng(jax.random.key(int.from_bytes(__import__("os").urandom(4), "little")))
    _w = (lambda a: (lambda t: t.astype(jnp.bfloat16) if jnp.issubdtype(t.dtype, jnp.floating) else t)(jnp.asarray(a)))
    def _A_setup():
        B, S, D, H = 1, 2048, 1024, 32
        Dh = D // H
        return {
            "x": _w((lambda *s: _rng.normal(s) * 0.05)(B, S, D)),
            "wq": _w((lambda *s: _rng.normal(s) * 1.6)(D, H * Dh)),
            "wk": _w((lambda *s: _rng.normal(s) * 1.6)(D, Dh)),
            "wv": _w((lambda *s: _rng.normal(s) * 0.1)(D, Dh)),
            "wo": _w((lambda *s: _rng.normal(s) * 0.1)(H * Dh, D)),
        }
    _A_in = _A_setup()

    def _B_setup():
        B, S, D = 1, 2048, 1024
        return {
            "x": _w((lambda *s: _rng.normal(s) * 0.2)(B, S, D)),
            "wqkv": _w((lambda *s: _rng.normal(s) * 0.2)(D, 3 * D)),
            "wo": _w((lambda *s: _rng.normal(s) * 0.05)(D, D)),
        }
    _B_in = _B_setup()

    return {
        "A_x": _A_in["x"],
        "A_wq": _A_in["wq"],
        "A_wk": _A_in["wk"],
        "A_wv": _A_in["wv"],
        "A_wo": _A_in["wo"],
        "B_x": _B_in["x"],
        "B_wqkv": _B_in["wqkv"],
        "B_wo": _B_in["wo"],
    }

def reference(A_x, A_wq, A_wk, A_wv, A_wo, B_x, B_wqkv, B_wo):
    def _A_ref(x, wq, wk, wv, wo):
        B, S, D = x.shape
        H = 32
        Dh = D // H
        q = (lambda x, *d: x.transpose(*d))((x @ wq).reshape(B, S, H, Dh), 0, 2, 1, 3)
        k = x @ wk
        v = x @ wv
        scores = jnp.einsum("bhqd,bkd->bhqk", q, k) * (Dh ** -0.5)
        p = _softmax(scores, axis=-1)
        o = jnp.einsum("bhqk,bkd->bhqd", p, v)
        return (lambda x, *d: x.transpose(*d))(o, 0, 2, 1, 3).reshape(B, S, H * Dh) @ wo

    def _B_ref(x, wqkv, wo):
        B, S, D = x.shape
        H = 32; Dh = D // H; W = 256
        qkv = (lambda x, *d: x.transpose(*d))((x @ wqkv).reshape(B, S, 3, H, Dh), 2, 0, 3, 1, 4)
        q, k, v = qkv[0], qkv[1], qkv[2]
        scores = jnp.einsum("bhqd,bhkd->bhqk", q, k) * (Dh ** -0.5)
        idx = jnp.arange(S)
        mask = (idx[:, None] - idx[None, :] >= 0) & (idx[:, None] - idx[None, :] < W)
        scores = jnp.where(mask[None, None], scores, -1e9)
        p = _softmax(scores, axis=-1)
        o = jnp.einsum("bhqk,bhkd->bhqd", p, v)
        return (lambda x, *d: x.transpose(*d))(o, 0, 2, 1, 3).reshape(B, S, D) @ wo

    a = _A_ref(A_x, A_wq, A_wk, A_wv, A_wo)
    b = _B_ref(B_x, B_wqkv, B_wo)
    return jnp.concatenate([a, b], axis=-1)
```

```python
import functools
import jax
import jax.numpy as jnp
from jax import lax
import jax.experimental.pallas as pl
import jax.experimental.pallas.tpu as pltpu

S = 2048
D = 1024
H = 32
DH = 32
W = 256
TQ = 256
TB = 128
KW = W + TB
LOG2E = 1.4426950408889634
QSCALE = (DH ** -0.5) * LOG2E
NEG = -1e9 * LOG2E
BF = jnp.bfloat16
F32 = jnp.float32


def _dot(a, b):
    return jnp.dot(a, b, preferred_element_type=F32)


def _kernel(xa_ref, wqa_ref, wka_ref, wva_ref, woa_ref, xb_ref, wqkv_ref, wob_ref, o_ref,
            ka_scr, vta_scr, qta_scr, ota_scr, sa_scr, sb_scr, ma_scr, mb_scr,
            kb_scr, vtb_scr, qtb_scr, otb_scr):
    i = pl.program_id(0)
    row0 = pl.multiple_of(i * TQ, TQ)

    @pl.when(i == 0)
    def _init():
        xa = xa_ref[...]
        ka_scr[...] = _dot(xa, wka_ref[...]).astype(BF)
        vta_scr[...] = _dot(xa, wva_ref[...]).T.astype(BF)
        kb_scr[0:W, :] = jnp.zeros((W, D), BF)
        vtb_scr[:, 0:W] = jnp.zeros((D, W), BF)

    qa = _dot(xa_ref[pl.ds(row0, TQ), :], wqa_ref[...]) * QSCALE
    qta_scr[...] = qa.T.astype(BF)

    def a_scores(h, s_ref, m_ref):
        qt = qta_scr[pl.ds(pl.multiple_of(h * DH, DH), DH), :]
        s = _dot(ka_scr[...], qt)
        s_ref[...] = s
        m_ref[...] = jnp.max(s, axis=0, keepdims=True)

    def a_out(h, s_ref, m_ref):
        p = jnp.exp2(s_ref[...] - m_ref[...])
        l = jnp.sum(p, axis=0, keepdims=True)
        ot = _dot(vta_scr[...], p.astype(BF))
        ota_scr[pl.ds(pl.multiple_of(h * DH, DH), DH), :] = ot / l

    a_scores(0, sa_scr, ma_scr)

    def a_body(j, carry):
        h = 2 * j
        a_scores(h + 1, sb_scr, mb_scr)
        a_out(h, sa_scr, ma_scr)
        a_scores(h + 2, sa_scr, ma_scr)
        a_out(h + 1, sb_scr, mb_scr)
        return carry

    lax.fori_loop(0, H // 2 - 1, a_body, 0)
    a_scores(H - 1, sb_scr, mb_scr)
    a_out(H - 2, sa_scr, ma_scr)
    a_out(H - 1, sb_scr, mb_scr)

    oa = ota_scr[...].T.astype(BF)
    o_ref[:, 0:D] = _dot(oa, woa_ref[...]).astype(o_ref.dtype)

    qkv = _dot(xb_ref[pl.ds(row0, TQ), :], wqkv_ref[...])
    qtb_scr[...] = (qkv[:, 0:D] * QSCALE).T.astype(BF)
    kb_scr[pl.ds(pl.multiple_of(row0 + W, TQ), TQ), :] = qkv[:, D:2 * D].astype(BF)
    vtb_scr[:, pl.ds(pl.multiple_of(row0 + W, TQ), TQ)] = qkv[:, 2 * D:3 * D].T.astype(BF)

    jr = lax.broadcasted_iota(jnp.int32, (KW, TB), 0)
    ir = lax.broadcasted_iota(jnp.int32, (KW, TB), 1)
    rowgrp = lax.broadcasted_iota(jnp.int32, (128, TB), 0) // DH
    masks = []
    for sub in range(TQ // TB):
        t0 = row0 + sub * TB
        lo = jnp.maximum(ir + 1, W - t0)
        masks.append((jr >= lo) & (jr <= ir + W))

    def b_body(c, carry):
        c0 = pl.multiple_of(c * 128, 128)
        for sub in range(TQ // TB):
            k0 = pl.multiple_of(row0 + sub * TB, TB)
            kwin = kb_scr[pl.ds(k0, KW), pl.ds(c0, 128)]
            qt = qtb_scr[pl.ds(c0, 128), sub * TB:(sub + 1) * TB]
            for j in range(4):
                qm = jnp.where(rowgrp == j, qt, jnp.zeros_like(qt))
                s = _dot(kwin, qm)
                s = jnp.where(masks[sub], s, NEG)
                m = jnp.max(s, axis=0, keepdims=True)
                p = jnp.exp2(s - m)
                l = jnp.sum(p, axis=0, keepdims=True)
                r0 = pl.multiple_of(c0 + j * DH, DH)
                vt = vtb_scr[pl.ds(r0, DH), pl.ds(k0, KW)]
                ot = _dot(vt, p.astype(BF))
                otb_scr[pl.ds(r0, DH), sub * TB:(sub + 1) * TB] = ot / l
        return carry

    lax.fori_loop(0, D // 128, b_body, 0)

    ob = otb_scr[...].T.astype(BF)
    o_ref[:, D:2 * D] = _dot(ob, wob_ref[...]).astype(o_ref.dtype)


@jax.jit
def pallas_concat_heads__grouped_kv_mqa__sliding_block__prompt_kernel(
    A_x, A_wq, A_wk, A_wv, A_wo, B_x, B_wqkv, B_wo):
    xa = A_x.reshape(S, D)
    xb = B_x.reshape(S, D)

    def full(shape):
        return pl.BlockSpec(shape, lambda i: (0,) * len(shape), pipeline_mode=pl.Buffered(1))

    out = pl.pallas_call(
        _kernel,
        grid=(S // TQ,),
        in_specs=[full((S, D)), full((D, D)), full((D, DH)), full((D, DH)), full((D, D)),
                  full((S, D)), full((D, 3 * D)), full((D, D))],
        out_specs=pl.BlockSpec((TQ, 2 * D), lambda i: (i, 0)),
        out_shape=jax.ShapeDtypeStruct((S, 2 * D), BF),
        scratch_shapes=[
            pltpu.VMEM((S, DH), BF),
            pltpu.VMEM((DH, S), BF),
            pltpu.VMEM((D, TQ), BF),
            pltpu.VMEM((D, TQ), F32),
            pltpu.VMEM((S, TQ), F32),
            pltpu.VMEM((S, TQ), F32),
            pltpu.VMEM((1, TQ), F32),
            pltpu.VMEM((1, TQ), F32),
            pltpu.VMEM((S + W, D), BF),
            pltpu.VMEM((D, S + W), BF),
            pltpu.VMEM((D, TQ), BF),
            pltpu.VMEM((D, TQ), F32),
        ],
        compiler_params=pltpu.CompilerParams(
            dimension_semantics=("arbitrary",),
            vmem_limit_bytes=100 * 1024 * 1024),
    )(xa, A_wq, A_wk, A_wv, A_wo, xb, B_wqkv, B_wo)
    return out.reshape(1, S, 2 * D)
```

```python
import jax
import jax.numpy as jnp
from jax import lax
import jax.experimental.pallas as pl
import jax.experimental.pallas.tpu as pltpu

S = 2048
D = 1024
H = 32
DH = 32
W = 256
TQ = 256
TB = 128
KW = W + TB
KC = 128
DELAY = 6
BH = (6, 14, 24)
XC = 512
NC = 256
RC = 512
LOG2E = 1.4426950408889634
QSCALE = (DH ** -0.5) * LOG2E
NEG = -1e9 * LOG2E
BF = jnp.bfloat16
F32 = jnp.float32
NUA = (S // TQ) * H
NIT = NUA // 2
NCH = S // KC
NLC = D // 128
assert NIT == (S // TB) * NLC


def _dot(a, b):
    return jnp.dot(a, b, preferred_element_type=F32)


def _kernel(xa_hbm, wqa_hbm, wka_hbm, wva_hbm, woa_hbm, xb_hbm, wqkv_hbm, wob_hbm, o_hbm,
            xa, wqa, wkv, woa, xb, wqkv, wob, out_v, isem, xsem, wsem, osem,
            ka, vta, qta, ota, sa, sb, ma, mb, kb, vtb, qtb, otb, bias):
    def xa_copy(r):
        rows = pl.ds(pl.multiple_of(r * XC, XC), XC)
        return pltpu.make_async_copy(xa_hbm.at[rows, :], xa.at[rows, :], xsem.at[r])

    cp_wk = pltpu.make_async_copy(wka_hbm, wkv.at[0:DH, :], isem.at[0])
    cp_wv = pltpu.make_async_copy(wva_hbm, wkv.at[DH:2 * DH, :], isem.at[1])
    cp_wq = [pltpu.make_async_copy(wqa_hbm.at[:, n * NC:(n + 1) * NC],
                                   wqa.at[:, n * NC:(n + 1) * NC], wsem.at[n])
             for n in range(D // NC)]
    cps = [pltpu.make_async_copy(s_, d_, isem.at[2 + n]) for n, (s_, d_) in enumerate(
        zip((xb_hbm, wqkv_hbm, woa_hbm, wob_hbm), (xb, wqkv, woa, wob)))]
    cp_wq[0].start()
    xa_copy(0).start()

    jr = lax.broadcasted_iota(jnp.int32, (KW, TB), 0)
    ir = lax.broadcasted_iota(jnp.int32, (KW, TB), 1)
    for v in range(3):
        lo = jnp.maximum(ir + 1, W - v * TB)
        ok = (jr >= lo) & (jr <= ir + W)
        bias[v] = jnp.where(ok, 0.0, NEG).astype(F32)
    kb[0:W, :] = jnp.zeros((W, D), BF)
    vtb[:, 0:W] = jnp.zeros((D, W), BF)

    cp_wq[0].wait()
    xa_copy(0).wait()
    for n in range(1, D // NC):
        cp_wq[n].start()
    for r in range(1, S // XC):
        xa_copy(r).start()
    cp_wk.start()
    cp_wv.start()
    for n in range(D // NC):
        if n > 0:
            cp_wq[n].wait()
        q = _dot(xa[0:XC, :], wqa[:, n * NC:(n + 1) * NC]) * QSCALE
        qta[n * NC:(n + 1) * NC, 0:XC] = q.T.astype(BF)

    def qa_body(r, c):
        xa_copy(r).wait()

        @pl.when(r == 1)
        def _():
            for c_ in cps:
                c_.start()
        r0 = pl.multiple_of(r * XC, XC)
        q = _dot(xa[pl.ds(r0, XC), :], wqa[...]) * QSCALE
        qta[:, pl.ds(r0, XC)] = q.T.astype(BF)
        return c
    lax.fori_loop(1, S // XC, qa_body, 0)

    cp_wk.wait()
    cp_wv.wait()
    kvt = lax.dot_general(wkv[...], xa[...], (((1,), (1,)), ((), ())),
                          preferred_element_type=F32)
    ka[...] = kvt[0:DH].T.astype(BF)
    vta[...] = kvt[DH:2 * DH].astype(BF)

    cps[0].wait()
    cps[1].wait()

    def qb_body(n, c):
        n0 = pl.multiple_of(n * NC, NC)
        q = _dot(xb[...], wqkv[:, pl.ds(n0, NC)]) * QSCALE
        qtb[pl.ds(n0, NC), :] = q.T.astype(BF)
        return c
    lax.fori_loop(0, D // NC, qb_body, 0)

    def kb_body(n, c):
        n0 = pl.multiple_of(n * NC, NC)
        k = _dot(xb[...], wqkv[:, pl.ds(pl.multiple_of(D + n0, NC), NC)])
        kb[W:W + S, pl.ds(n0, NC)] = k.astype(BF)
        return c
    lax.fori_loop(0, D // NC, kb_body, 0)

    def vb_body(n, c):
        n0 = pl.multiple_of(n * NC, NC)
        v = _dot(xb[...], wqkv[:, pl.ds(pl.multiple_of(2 * D + n0, NC), NC)])
        vtb[pl.ds(n0, NC), W:W + S] = v.T.astype(BF)
        return c
    lax.fori_loop(0, D // NC, vb_body, 0)

    def a_stream(u, hooks):
        bufs = ((sa, ma, sb, mb), (sb, mb, sa, ma))
        st = [dict(mx=None, l=None, acc=None) for _ in range(2)]
        pend = []

        def pv():
            j, kc, pb = pend.pop(0)
            d = _dot(vta[:, kc * KC:(kc + 1) * KC], pb)
            z = st[j]
            z["acc"] = d if z["acc"] is None else z["acc"] + d
            if kc == NCH - 1:
                uu = u + j
                q0 = pl.multiple_of((uu // H) * TQ, TQ)
                r0 = pl.multiple_of((uu % H) * DH, DH)
                ota[pl.ds(r0, DH), pl.ds(q0, TQ)] = z["acc"] * (1.0 / z["l"])

        for j in range(2):
            cur, mcur, nxt, mnxt = bufs[j]
            z = st[j]
            un = jnp.minimum(u + j + 1, NUA - 1)
            qn0 = pl.multiple_of((un // H) * TQ, TQ)
            rn0 = pl.multiple_of((un % H) * DH, DH)
            qt = qta[pl.ds(rn0, DH), pl.ds(qn0, TQ)]
            m = mcur[...]
            for kc in range(NCH):
                rows = slice(kc * KC, (kc + 1) * KC)
                sn = _dot(ka[rows, :], qt)
                nxt[rows, :] = sn
                mc = jnp.max(sn, axis=0, keepdims=True)
                z["mx"] = mc if z["mx"] is None else jnp.maximum(z["mx"], mc)
                p = jnp.exp2(cur[rows, :] - m)
                lc = jnp.sum(p, axis=0, keepdims=True)
                z["l"] = lc if z["l"] is None else z["l"] + lc
                pend.append((j, kc, p.astype(BF)))
                if len(pend) > DELAY:
                    pv()
                t = j * NCH + kc
                if t in hooks:
                    hooks[t]()
            mnxt[...] = z["mx"]
        while pend:
            pv()

    rowgrp = lax.broadcasted_iota(jnp.int32, (128, TB), 0) // DH

    def b_stages(b):
        st = b // NLC
        c0 = pl.multiple_of((b % NLC) * 128, 128)
        k0 = pl.multiple_of(st * TB, TB)
        state = {}

        def stage1():
            kwin = kb[pl.ds(k0, KW), pl.ds(c0, 128)]
            qt = qtb[pl.ds(c0, 128), pl.ds(k0, TB)]
            q4 = jnp.concatenate(
                [jnp.where(rowgrp == j, qt, jnp.zeros_like(qt)) for j in range(4)], axis=1)
            bs = bias[jnp.minimum(st, 2)]
            bs = jnp.concatenate([bs] * 4, axis=1)
            s = _dot(kwin, q4)
            s = jnp.where(bs < 0.0, bs, s)
            state["s"] = s
            state["m"] = jnp.max(s, axis=0, keepdims=True)

        def stage2():
            p = jnp.exp2(state["s"] - state["m"])
            l = jnp.sum(p, axis=0, keepdims=True)
            state["p"] = p.astype(BF)
            state["rl"] = 1.0 / l

        def stage3():
            pb, rl = state["p"], state["rl"]
            for j in range(4):
                r0 = pl.multiple_of(c0 + j * DH, DH)
                vt = vtb[pl.ds(r0, DH), pl.ds(k0, KW)]
                ot = _dot(vt, pb[:, j * TB:(j + 1) * TB])
                otb[pl.ds(r0, DH), pl.ds(k0, TB)] = ot * rl[:, j * TB:(j + 1) * TB]

        return stage1, stage2, stage3

    def body(it, c):
        b1, b2, b3 = b_stages(it)
        a_stream(2 * it, {BH[0]: b1, BH[1]: b2, BH[2]: b3})
        return c

    s_first = _dot(ka[...], qta[0:DH, 0:TQ])
    sa[...] = s_first
    ma[...] = jnp.max(s_first, axis=0, keepdims=True)
    lax.fori_loop(0, NIT, body, 0)

    cps[2].wait()
    cps[3].wait()

    def o_copy(r):
        rows = pl.ds(pl.multiple_of(r * RC, RC), RC)
        return pltpu.make_async_copy(out_v.at[rows, :], o_hbm.at[rows, :], osem.at[r])

    def o_body(r, c):
        rows = pl.ds(pl.multiple_of(r * RC, RC), RC)
        out_v[rows, 0:D] = _dot(ota[:, rows].T.astype(BF), woa[...]).astype(BF)
        out_v[rows, D:2 * D] = _dot(otb[:, rows].T.astype(BF), wob[...]).astype(BF)
        o_copy(r).start()
        return c
    lax.fori_loop(0, S // RC, o_body, 0)
    for r in range(S // RC):
        o_copy(r).wait()


@jax.jit
def pallas_concat_heads__grouped_kv_mqa__sliding_block__prompt_kernel(
    A_x: jax.Array,
    A_wq: jax.Array,
    A_wk: jax.Array,
    A_wv: jax.Array,
    A_wo: jax.Array,
    B_x: jax.Array,
    B_wqkv: jax.Array,
    B_wo: jax.Array,
):
    xa = A_x.reshape(S, D)
    xb = B_x.reshape(S, D)
    anyspec = pl.BlockSpec(memory_space=pl.ANY)
    out = pl.pallas_call(
        _kernel,
        in_specs=[anyspec] * 8,
        out_specs=anyspec,
        out_shape=jax.ShapeDtypeStruct((S, 2 * D), BF),
        scratch_shapes=[
            pltpu.VMEM((S, D), BF),
            pltpu.VMEM((D, D), BF),
            pltpu.VMEM((2 * DH, D), BF),
            pltpu.VMEM((D, D), BF),
            pltpu.VMEM((S, D), BF),
            pltpu.VMEM((D, 3 * D), BF),
            pltpu.VMEM((D, D), BF),
            pltpu.VMEM((S, 2 * D), BF),
            pltpu.SemaphoreType.DMA((6,)),
            pltpu.SemaphoreType.DMA((S // XC,)),
            pltpu.SemaphoreType.DMA((D // NC,)),
            pltpu.SemaphoreType.DMA((S // RC,)),
            pltpu.VMEM((S, DH), BF),
            pltpu.VMEM((DH, S), BF),
            pltpu.VMEM((D, S), BF),
            pltpu.VMEM((D, S), F32),
            pltpu.VMEM((S, TQ), F32),
            pltpu.VMEM((S, TQ), F32),
            pltpu.VMEM((1, TQ), F32),
            pltpu.VMEM((1, TQ), F32),
            pltpu.VMEM((S + W, D), BF),
            pltpu.VMEM((D, S + W), BF),
            pltpu.VMEM((D, S), BF),
            pltpu.VMEM((D, S), F32),
            pltpu.VMEM((3, KW, TB), F32),
        ],
        compiler_params=pltpu.CompilerParams(vmem_limit_bytes=110 * 1024 * 1024),
    )(xa, A_wq, A_wk.T, A_wv.T, A_wo, xb, B_wqkv, B_wo)
    return out.reshape(1, S, 2 * D)
```

```python
import jax
import jax.numpy as jnp
from jax import lax
import jax.experimental.pallas as pl
import jax.experimental.pallas.tpu as pltpu

S = 2048
D = 1024
H = 32
DH = 32
W = 256
TQ = 256
TB = 128
KW = W + TB
KC = 128
DELAY = 6
BH = (6, 14, 24)
XC = 512
NC = 256
RC = 512
LOG2E = 1.4426950408889634
QSCALE = (DH ** -0.5) * LOG2E
NEG = -1e9 * LOG2E
BF = jnp.bfloat16
F32 = jnp.float32
NUA = (S // TQ) * H
NIT = NUA // 2
NCH = S // KC
NLC = D // 128
assert NIT == (S // TB) * NLC


def _dot(a, b):
    return jnp.dot(a, b, preferred_element_type=F32)


def _kernel(xa_hbm, wqa_hbm, wka_hbm, wva_hbm, woa_hbm, xb_hbm, wqkv_hbm, wob_hbm, o_hbm,
            xa, wqa, wkv, woa, xb, wqkv, wob, out_v, isem, xsem, wsem, osem,
            ka, vta, qta, ota, sa, sb, ma, mb, kb, vtb, qtb, otb, bias):
    def xa_copy(r):
        rows = pl.ds(pl.multiple_of(r * XC, XC), XC)
        return pltpu.make_async_copy(xa_hbm.at[rows, :], xa.at[rows, :], xsem.at[r])

    cp_wk = pltpu.make_async_copy(wka_hbm, wkv.at[0:DH, :], isem.at[0])
    cp_wv = pltpu.make_async_copy(wva_hbm, wkv.at[DH:2 * DH, :], isem.at[1])
    cp_wq = [pltpu.make_async_copy(wqa_hbm.at[:, n * NC:(n + 1) * NC],
                                   wqa.at[:, n * NC:(n + 1) * NC], wsem.at[n])
             for n in range(D // NC)]
    cps = [pltpu.make_async_copy(s_, d_, isem.at[2 + n]) for n, (s_, d_) in enumerate(
        zip((xb_hbm, wqkv_hbm, woa_hbm, wob_hbm), (xb, wqkv, woa, wob)))]
    cp_wq[0].start()
    xa_copy(0).start()

    jr = lax.broadcasted_iota(jnp.int32, (KW, TB), 0)
    ir = lax.broadcasted_iota(jnp.int32, (KW, TB), 1)
    for v in range(3):
        lo = jnp.maximum(ir + 1, W - v * TB)
        ok = (jr >= lo) & (jr <= ir + W)
        bias[v] = jnp.where(ok, 0.0, NEG).astype(F32)
    kb[0:W, :] = jnp.zeros((W, D), BF)
    vtb[:, 0:W] = jnp.zeros((D, W), BF)

    cp_wq[0].wait()
    xa_copy(0).wait()
    for n in range(1, D // NC):
        cp_wq[n].start()
    for r in range(1, S // XC):
        xa_copy(r).start()
    cp_wk.start()
    cp_wv.start()
    for n in range(D // NC):
        if n > 0:
            cp_wq[n].wait()
        q = _dot(xa[0:XC, :], wqa[:, n * NC:(n + 1) * NC]) * QSCALE
        qta[n * NC:(n + 1) * NC, 0:XC] = q.T.astype(BF)

    def qa_body(r, c):
        xa_copy(r).wait()

        @pl.when(r == 1)
        def _():
            for c_ in cps:
                c_.start()
        r0 = pl.multiple_of(r * XC, XC)
        q = _dot(xa[pl.ds(r0, XC), :], wqa[...]) * QSCALE
        qta[:, pl.ds(r0, XC)] = q.T.astype(BF)
        return c
    lax.fori_loop(1, S // XC, qa_body, 0)

    cp_wk.wait()
    cp_wv.wait()
    kvt = lax.dot_general(wkv[...], xa[...], (((1,), (1,)), ((), ())),
                          preferred_element_type=F32)
    ka[...] = kvt[0:DH].T.astype(BF)
    vta[...] = kvt[DH:2 * DH].astype(BF)

    cps[0].wait()
    cps[1].wait()

    def qb_body(n, c):
        n0 = pl.multiple_of(n * NC, NC)
        q = _dot(xb[...], wqkv[:, pl.ds(n0, NC)]) * QSCALE
        qtb[pl.ds(n0, NC), :] = q.T.astype(BF)
        return c
    lax.fori_loop(0, D // NC, qb_body, 0)

    def kb_body(n, c):
        n0 = pl.multiple_of(n * NC, NC)
        k = _dot(xb[...], wqkv[:, pl.ds(pl.multiple_of(D + n0, NC), NC)])
        kb[W:W + S, pl.ds(n0, NC)] = k.astype(BF)
        return c
    lax.fori_loop(0, D // NC, kb_body, 0)

    def vb_body(n, c):
        n0 = pl.multiple_of(n * NC, NC)
        v = _dot(xb[...], wqkv[:, pl.ds(pl.multiple_of(2 * D + n0, NC), NC)])
        vtb[pl.ds(n0, NC), W:W + S] = v.T.astype(BF)
        return c
    lax.fori_loop(0, D // NC, vb_body, 0)

    def a_stream(u, hooks):
        bufs = ((sa, ma, sb, mb), (sb, mb, sa, ma))
        st = [dict(mx=None, l=None, acc=None) for _ in range(2)]
        pend = []

        def pv():
            j, kc, pb = pend.pop(0)
            d = _dot(vta[:, kc * KC:(kc + 1) * KC], pb)
            z = st[j]
            z["acc"] = d if z["acc"] is None else z["acc"] + d
            if kc == NCH - 1:
                uu = u + j
                q0 = pl.multiple_of((uu // H) * TQ, TQ)
                r0 = pl.multiple_of((uu % H) * DH, DH)
                l = jnp.sum(z["l"], axis=0, keepdims=True)
                ota[pl.ds(r0, DH), pl.ds(q0, TQ)] = z["acc"] * (1.0 / l)

        for j in range(2):
            cur, mcur, nxt, mnxt = bufs[j]
            z = st[j]
            un = jnp.minimum(u + j + 1, NUA - 1)
            qn0 = pl.multiple_of((un // H) * TQ, TQ)
            rn0 = pl.multiple_of((un % H) * DH, DH)
            qt = qta[pl.ds(rn0, DH), pl.ds(qn0, TQ)]
            m = mcur[...]
            for kc in range(NCH):
                rows = slice(kc * KC, (kc + 1) * KC)
                sn = _dot(ka[rows, :], qt)
                nxt[rows, :] = sn
                mc = jnp.max(sn.reshape(KC // 8, 8, TQ), axis=0)
                z["mx"] = mc if z["mx"] is None else jnp.maximum(z["mx"], mc)
                p = jnp.exp2(cur[rows, :] - m)
                lc = jnp.sum(p.reshape(KC // 8, 8, TQ), axis=0)
                z["l"] = lc if z["l"] is None else z["l"] + lc
                pend.append((j, kc, p.astype(BF)))
                if len(pend) > DELAY:
                    pv()
                t = j * NCH + kc
                if t in hooks:
                    hooks[t]()
            mnxt[...] = jnp.max(z["mx"], axis=0, keepdims=True)
        while pend:
            pv()

    rowgrp = lax.broadcasted_iota(jnp.int32, (128, TB), 0) // DH

    def b_stages(b):
        st = b // NLC
        c0 = pl.multiple_of((b % NLC) * 128, 128)
        k0 = pl.multiple_of(st * TB, TB)
        state = {}

        def stage1():
            kwin = kb[pl.ds(k0, KW), pl.ds(c0, 128)]
            qt = qtb[pl.ds(c0, 128), pl.ds(k0, TB)]
            q4 = jnp.concatenate(
                [jnp.where(rowgrp == j, qt, jnp.zeros_like(qt)) for j in range(4)], axis=1)
            bs = bias[jnp.minimum(st, 2)]
            bs = jnp.concatenate([bs] * 4, axis=1)
            s = _dot(kwin, q4)
            s = jnp.where(bs < 0.0, bs, s)
            state["s"] = s
            state["m"] = jnp.max(s, axis=0, keepdims=True)

        def stage2():
            p = jnp.exp2(state["s"] - state["m"])
            l = jnp.sum(p, axis=0, keepdims=True)
            state["p"] = p.astype(BF)
            state["rl"] = 1.0 / l

        def stage3():
            pb, rl = state["p"], state["rl"]
            for j in range(4):
                r0 = pl.multiple_of(c0 + j * DH, DH)
                vt = vtb[pl.ds(r0, DH), pl.ds(k0, KW)]
                ot = _dot(vt, pb[:, j * TB:(j + 1) * TB])
                otb[pl.ds(r0, DH), pl.ds(k0, TB)] = ot * rl[:, j * TB:(j + 1) * TB]

        return stage1, stage2, stage3

    def body(it, c):
        b1, b2, b3 = b_stages(it)
        a_stream(2 * it, {BH[0]: b1, BH[1]: b2, BH[2]: b3})
        return c

    s_first = _dot(ka[...], qta[0:DH, 0:TQ])
    sa[...] = s_first
    ma[...] = jnp.max(s_first, axis=0, keepdims=True)
    lax.fori_loop(0, NIT, body, 0)

    cps[2].wait()
    cps[3].wait()

    def o_copy(r):
        rows = pl.ds(pl.multiple_of(r * RC, RC), RC)
        return pltpu.make_async_copy(out_v.at[rows, :], o_hbm.at[rows, :], osem.at[r])

    def o_body(r, c):
        rows = pl.ds(pl.multiple_of(r * RC, RC), RC)
        out_v[rows, 0:D] = _dot(ota[:, rows].T.astype(BF), woa[...]).astype(BF)
        out_v[rows, D:2 * D] = _dot(otb[:, rows].T.astype(BF), wob[...]).astype(BF)
        o_copy(r).start()
        return c
    lax.fori_loop(0, S // RC, o_body, 0)
    for r in range(S // RC):
        o_copy(r).wait()


@jax.jit
def pallas_concat_heads__grouped_kv_mqa__sliding_block__prompt_kernel(
    A_x: jax.Array,
    A_wq: jax.Array,
    A_wk: jax.Array,
    A_wv: jax.Array,
    A_wo: jax.Array,
    B_x: jax.Array,
    B_wqkv: jax.Array,
    B_wo: jax.Array,
):
    xa = A_x.reshape(S, D)
    xb = B_x.reshape(S, D)
    anyspec = pl.BlockSpec(memory_space=pl.ANY)
    out = pl.pallas_call(
        _kernel,
        in_specs=[anyspec] * 8,
        out_specs=anyspec,
        out_shape=jax.ShapeDtypeStruct((S, 2 * D), BF),
        scratch_shapes=[
            pltpu.VMEM((S, D), BF),
            pltpu.VMEM((D, D), BF),
            pltpu.VMEM((2 * DH, D), BF),
            pltpu.VMEM((D, D), BF),
            pltpu.VMEM((S, D), BF),
            pltpu.VMEM((D, 3 * D), BF),
            pltpu.VMEM((D, D), BF),
            pltpu.VMEM((S, 2 * D), BF),
            pltpu.SemaphoreType.DMA((6,)),
            pltpu.SemaphoreType.DMA((S // XC,)),
            pltpu.SemaphoreType.DMA((D // NC,)),
            pltpu.SemaphoreType.DMA((S // RC,)),
            pltpu.VMEM((S, DH), BF),
            pltpu.VMEM((DH, S), BF),
            pltpu.VMEM((D, S), BF),
            pltpu.VMEM((D, S), F32),
            pltpu.VMEM((S, TQ), F32),
            pltpu.VMEM((S, TQ), F32),
            pltpu.VMEM((1, TQ), F32),
            pltpu.VMEM((1, TQ), F32),
            pltpu.VMEM((S + W, D), BF),
            pltpu.VMEM((D, S + W), BF),
            pltpu.VMEM((D, S), BF),
            pltpu.VMEM((D, S), F32),
            pltpu.VMEM((3, KW, TB), F32),
        ],
        compiler_params=pltpu.CompilerParams(vmem_limit_bytes=110 * 1024 * 1024),
    )(xa, A_wq, A_wk.T, A_wv.T, A_wo, xb, B_wqkv, B_wo)
    return out.reshape(1, S, 2 * D)
```
